```python
import os as _os
_os.environ.setdefault("JAX_PLATFORMS", "cpu")
import jax
import jax.numpy as jnp

def _softmax(x, axis=-1):
    return jax.nn.softmax(x, axis=axis)
def _gelu(x):
    return jax.nn.gelu(x, approximate=True)
def _silu(x):
    return jax.nn.silu(x)
def _sigmoid(x):
    return jax.nn.sigmoid(x)
def _layernorm(x, axis=-1, eps=1e-5):
    m = jnp.mean(x, axis=axis, keepdims=True)
    v = jnp.var(x, axis=axis, keepdims=True)
    return (x - m) / jnp.sqrt(v + eps)
def _scatter_add(tgt, idx, src, axis=0):
    return tgt.at[idx].add(src)
def _segment_sum(src, seg, n):
    return jax.ops.segment_sum(src, seg, n)
class _Rng:
    def __init__(self, key):
        self._k = key
    def _next(self):
        self._k, sub = jax.random.split(self._k)
        return sub
    def normal(self, shape):
        return jax.random.normal(self._next(), shape, dtype=jnp.bfloat16)
    def randint(self, lo, hi, shape):
        return jax.random.randint(self._next(), shape, lo, hi, dtype=jnp.int32)
    def uniform(self, shape, lo=0.0, hi=1.0):
        return jax.random.uniform(self._next(), shape, jnp.bfloat16, lo, hi)
    def permutation(self, n):
        return jax.random.permutation(self._next(), n)


kernel_name = 'gated_mix__sliding_block_cached__dense_activation_silu__decode'

def setup_inputs():
    _rng = _Rng(jax.random.key(int.from_bytes(__import__("os").urandom(4), "little")))
    _w = (lambda a: (lambda t: t.astype(jnp.bfloat16) if jnp.issubdtype(t.dtype, jnp.floating) else t)(jnp.asarray(a)))
    def _A_setup():
        B, Sq, D = 2, 1, 1024
        Hq, Hkv, Sk, Dh = 32, 4, 32768, 128
        assert Hq % Hkv == 0, (Hq, Hkv)
        return {
            "x": _w((lambda *s: _rng.normal(s) * 0.05)(B, Sq, D)),
            "k_cache": _w((lambda *s: _rng.normal(s) * 3.2)(B, Hkv, Sk, Dh)),
            "v_cache": _w((lambda *s: _rng.normal(s) * 0.05)(B, Hkv, Sk, Dh)),
            "wq": _w((lambda *s: _rng.normal(s) * 3.2)(D, Hq * Dh) * (D ** -0.5)),
            "wo": _w((lambda *s: _rng.normal(s) * 0.05)(Hq * Dh, D) * ((Hq * Dh) ** -0.5)),
        }
    _A_in = _A_setup()

    def _B_setup():
        B, S, D, F = 2, 1, 1024, 3584
        return {
            "x": _w((lambda *s: _rng.normal(s) * 0.05)(B, S, D)),
            "w1": _w((lambda *s: _rng.normal(s) * 0.05)(D, F) * (D ** -0.5)),
            "w2": _w((lambda *s: _rng.normal(s) * 0.05)(F, D) * (F ** -0.5)),
        }
    _B_in = _B_setup()

    return {
        "A_x": _A_in["x"],
        "A_k_cache": _A_in["k_cache"],
        "A_v_cache": _A_in["v_cache"],
        "A_wq": _A_in["wq"],
        "A_wo": _A_in["wo"],
        "B_x": _B_in["x"],
        "B_w1": _B_in["w1"],
        "B_w2": _B_in["w2"],
        "gate_w": _w((lambda *s: _rng.normal(s) * 0.05)(1024) * 16.0),
    }

def reference(A_x, A_k_cache, A_v_cache, A_wq, A_wo, B_x, B_w1, B_w2, gate_w):
    def _A_ref(x, k_cache, v_cache, wq, wo):
        B, Sq, D = x.shape
        Hq, Dh = 32, 128
        Hkv, Sk = k_cache.shape[1], k_cache.shape[2]
        W = min(4096, max(256, Sk // 4))
        rep = Hq // Hkv
        q = (lambda x, *d: x.transpose(*d))((x @ wq).reshape(B, Sq, Hq, Dh), 0, 2, 1, 3)
        k = jnp.repeat(k_cache[:, :, Sk - W:, :], rep, axis=1)
        v = jnp.repeat(v_cache[:, :, Sk - W:, :], rep, axis=1)
        scores = jnp.einsum("bhqd,bhkd->bhqk", q, k) * (Dh ** -0.5)
        p = _softmax(scores, axis=-1)
        o = jnp.einsum("bhqk,bhkd->bhqd", p, v)
        return (lambda x, *d: x.transpose(*d))(o, 0, 2, 1, 3).reshape(B, Sq, Hq * Dh) @ wo

    def _B_ref(x, w1, w2):
        h = jnp.einsum("bsd,df->bsf", x, w1)
        h = _silu(h)
        out = jnp.einsum("bsf,fd->bsd", h, w2)
        return out

    x = A_x
    g = _sigmoid((x * gate_w).sum(-1, keepdims=True))
    a = _A_ref(x, A_k_cache, A_v_cache, A_wq, A_wo)
    b = _B_ref(x, B_w1, B_w2)
    return g * a + (1 - g) * b
```

```python
import jax
import jax.numpy as jnp
from jax import lax
import jax.experimental.pallas as pl
import jax.experimental.pallas.tpu as pltpu

B, D = 2, 1024
HQ, HKV, DH = 32, 4, 128
REP = HQ // HKV
F = 3584
WO_CHUNKS = (2560, 1024, 384, 128)
assert sum(WO_CHUNKS) == HQ * DH


@jax.jit
def pallas_gated_mix__sliding_block_cached__dense_activation_silu__decode_kernel(
    A_x, A_k_cache, A_v_cache, A_wq, A_wo, B_x, B_w1, B_w2, gate_w,
):
    Sk = A_k_cache.shape[2]
    W = min(4096, max(256, Sk // 4))
    scale = DH ** -0.5

    def kernel(x_hbm, k_hbm, v_hbm, wq_hbm, wo_hbm, w1_hbm, w2_hbm, g_hbm, o_hbm,
               x_v, g_v, wq_v, k_v, v_v, wo_v, w1_v, w2_v, q_s, p_s, o_s, acc_s, out_v, sems):
        copies = {}
        order = []
        def add(name, src, dst):
            idx = len(order)
            copies[name] = pltpu.make_async_copy(src, dst, sems.at[idx])
            order.append(name)
        add('wq', wq_hbm, wq_v)
        add('x', x_hbm, x_v)
        add('g', g_hbm, g_v)
        add('k', k_hbm.at[:, :, pl.ds(Sk - W, W), :], k_v)
        add('v', v_hbm.at[:, :, pl.ds(Sk - W, W), :], v_v)
        add('w1', w1_hbm, w1_v)
        add('w2', w2_hbm, w2_v)
        r = 0
        for c, n in enumerate(WO_CHUNKS):
            add(('wo', c), wo_hbm.at[pl.ds(r, n), :], wo_v.at[pl.ds(r, n), :])
            r += n
        for n in order:
            copies[n].start()
        wait = lambda n: copies[n].wait()

        wait('x')
        wait('g')
        x2 = x_v[...]
        x2f = x2.astype(jnp.float32)
        gw = g_v[...].astype(jnp.float32).reshape(1, D)
        gate = jax.nn.sigmoid(jnp.sum(x2f * gw, axis=-1, keepdims=True))

        wait('wq')
        for g in range(HKV):
            qg = jnp.dot(x2, wq_v[:, pl.ds(g * REP * DH, REP * DH)], preferred_element_type=jnp.float32)
            for b in range(B):
                for h in range(REP):
                    q_s[b * HKV + g, pl.ds(h, 1), :] = qg[b:b + 1, h * DH:(h + 1) * DH]

        wait('k')
        ls = []
        for b in range(B):
            for g in range(HKV):
                i = b * HKV + g
                q = q_s[i].astype(jnp.bfloat16)
                s = lax.dot_general(q, k_v[b, g], (((1,), (1,)), ((), ())),
                                    preferred_element_type=jnp.float32) * scale
                m = jnp.max(s, axis=-1, keepdims=True)
                p = jnp.exp(s - m)
                ls.append(jnp.sum(p, axis=-1, keepdims=True))
                p_s[i] = p
        wait('v')
        for b in range(B):
            for g in range(HKV):
                i = b * HKV + g
                o = jnp.dot(p_s[i].astype(jnp.bfloat16), v_v[b, g], preferred_element_type=jnp.float32)
                o = o / ls[i]
                for h in range(REP):
                    hh = g * REP + h
                    o_s[pl.ds(b, 1), pl.ds(hh * DH, DH)] = o[h:h + 1, :]

        wait('w1')
        h = jnp.dot(x2, w1_v[...], preferred_element_type=jnp.float32)
        h = (h * jax.nn.sigmoid(h)).astype(jnp.bfloat16)
        wait('w2')
        bacc = jnp.dot(h, w2_v[...], preferred_element_type=jnp.float32)
        bterm = (1.0 - gate) * bacc

        o2 = o_s[...].astype(jnp.bfloat16)
        acc_s[...] = bterm
        r = 0
        for c, n in enumerate(WO_CHUNKS):
            wait(('wo', c))
            t = jnp.dot(o2[:, r:r + n], wo_v[pl.ds(r, n), :], preferred_element_type=jnp.float32)
            res = acc_s[...] + gate * t
            if c + 1 < len(WO_CHUNKS):
                acc_s[...] = res
            r += n
        out_v[...] = res.astype(jnp.bfloat16)
        oc = pltpu.make_async_copy(out_v, o_hbm, sems.at[0])
        oc.start()
        oc.wait()

    nsem = 7 + len(WO_CHUNKS)
    anyspec = pl.BlockSpec(memory_space=pl.ANY)
    out = pl.pallas_call(
        kernel,
        out_shape=jax.ShapeDtypeStruct((B, D), jnp.bfloat16),
        in_specs=[anyspec] * 8,
        out_specs=anyspec,
        scratch_shapes=[
            pltpu.VMEM((B, D), jnp.bfloat16),
            pltpu.VMEM((D,), jnp.bfloat16),
            pltpu.VMEM((D, HQ * DH), jnp.bfloat16),
            pltpu.VMEM((B, HKV, W, DH), jnp.bfloat16),
            pltpu.VMEM((B, HKV, W, DH), jnp.bfloat16),
            pltpu.VMEM((HQ * DH, D), jnp.bfloat16),
            pltpu.VMEM((D, F), jnp.bfloat16),
            pltpu.VMEM((F, D), jnp.bfloat16),
            pltpu.VMEM((B * HKV, REP, DH), jnp.float32),
            pltpu.VMEM((B * HKV, REP, W), jnp.float32),
            pltpu.VMEM((B, HQ * DH), jnp.float32),
            pltpu.VMEM((B, D), jnp.float32),
            pltpu.VMEM((B, D), jnp.bfloat16),
            pltpu.SemaphoreType.DMA((nsem,)),
        ],
        compiler_params=pltpu.CompilerParams(vmem_limit_bytes=100 * 1024 * 1024),
    )(A_x.reshape(B, D), A_k_cache, A_v_cache, A_wq, A_wo, B_w1, B_w2, gate_w)
    return out.reshape(B, 1, D)
```

```python
import jax
import jax.numpy as jnp
from jax import lax
import jax.experimental.pallas as pl
import jax.experimental.pallas.tpu as pltpu

HQ, DH = 32, 128
W_FG = 12
W_BG = 12
EARLY = 4
WO_FG = 256
BUDGET = 200
KT = 1024
NSP = 2
VPU_ROWS = 64
VPU_CHUNK = 32
LAST_ROWS = 32
LAST_CHUNK = 16


@jax.jit
def pallas_gated_mix__sliding_block_cached__dense_activation_silu__decode_kernel(
    A_x: jax.Array,
    A_k_cache: jax.Array,
    A_v_cache: jax.Array,
    A_wq: jax.Array,
    A_wo: jax.Array,
    B_x: jax.Array,
    B_w1: jax.Array,
    B_w2: jax.Array,
    gate_w: jax.Array,
):
    del B_x
    B, _, D = A_x.shape
    HKV, Sk = A_k_cache.shape[1], A_k_cache.shape[2]
    F = B_w1.shape[1]
    REP = HQ // HKV
    QD = HQ * DH
    W = min(4096, max(256, Sk // 4))
    scale = DH ** -0.5
    NKT = W // KT
    NS = D // 128
    bf16, f32 = jnp.bfloat16, jnp.float32
    heads = [(b, g) for g in range(HKV) for b in range(B)]

    def kernel(x_hbm, k_hbm, v_hbm, wq_hbm, wo_hbm, w1_hbm, w2_hbm, g_hbm, o_hbm,
               x_v, g_v, wq_v, k_v, v_v, wo_v, w1_v, w2_v,
               h_acc, h_s, q_acc, q_s, p_s, l_s, o_acc, o_s, acc_s, oc_s, out_v,
               sem_f, sem_b, sem_m):
        def rows(key, src, dst, lo, hi, n, csplit=1):
            out = []
            cw = src.shape[1] // csplit
            for r in range(lo, hi, n):
                for c in range(csplit):
                    if csplit == 1:
                        s_, d_ = src.at[pl.ds(r, n), :], dst.at[pl.ds(r, n), :]
                    else:
                        s_ = src.at[pl.ds(r, n), pl.ds(c * cw, cw)]
                        d_ = dst.at[pl.ds(r, n), pl.ds(c * cw, cw)]
                    out.append((s_, d_, key, r, r + n))
            return out

        def kv_rows(key, src, dst, n):
            return [(src.at[b, g, pl.ds(Sk - W + r, n), :], dst.at[b, g, pl.ds(r, n), :],
                     (key, b, g), r, r + n)
                    for (b, g) in heads for r in range(0, W, n)]

        bg = (rows('wq', wq_hbm, wq_v, 0, D, 8)
              + kv_rows('k', k_hbm, k_v, 256)
              + kv_rows('v', v_hbm, v_v, 256)
              + rows('wo', wo_hbm, wo_v, WO_FG, QD - LAST_ROWS, 32)
              + rows('wo', wo_hbm, wo_v, QD - LAST_ROWS, QD, LAST_CHUNK))
        fg = (rows('w1', w1_hbm, w1_v, 0, D, 8, csplit=2)
              + rows('w2', w2_hbm, w2_v, 0, F, 16)
              + rows('wo', wo_hbm, wo_v, 0, WO_FG, 16))
        NB, NF = len(bg), len(fg)

        def ready_of(key, lo, hi):
            hit = lambda e: e[2] == key and e[3] < hi and e[4] > lo
            return max([0] + [j for j, e in enumerate(bg) if hit(e)]
                       + [j - EARLY for j, e in enumerate(fg) if hit(e)])

        def cp_b(j):
            return pltpu.make_async_copy(bg[j][0], bg[j][1], sem_b.at[j % W_BG])

        def cp_f(j):
            return pltpu.make_async_copy(fg[j][0], fg[j][1], sem_f.at[j % W_FG])

        cx = pltpu.make_async_copy(x_hbm, x_v, sem_m.at[0])
        cg = pltpu.make_async_copy(g_hbm, g_v, sem_m.at[1])
        cx.start(priority=0)
        cg.start(priority=0)
        for j in range(W_BG):
            cp_b(j).start(priority=1)
        for j in range(W_FG):
            cp_f(j).start(priority=0)

        st = {}

        def t_init():
            cx.wait()
            cg.wait()
            gw = g_v[...].astype(f32).reshape(1, D)
            st['gate'] = jax.nn.sigmoid(
                jnp.sum(x_v[...].astype(f32) * gw, axis=-1, keepdims=True))

        def t_proj(s, c0, cw, w_v, acc, fin):
            def f():
                t = jnp.dot(x_v[:, pl.ds(s * 128, 128)], w_v[pl.ds(s * 128, 128), pl.ds(c0, cw)],
                            preferred_element_type=f32)
                if s == 0:
                    acc[:, pl.ds(c0, cw)] = t
                elif s < NS - 1:
                    acc[:, pl.ds(c0, cw)] += t
                else:
                    fin(acc[:, pl.ds(c0, cw)] + t, c0, cw)
            return f

        def fin_h(h, c0, cw):
            h_s[:, pl.ds(c0, cw)] = (h * jax.nn.sigmoid(h)).astype(bf16)

        def fin_q(q, c0, cw):
            for b in range(B):
                for hh in range(c0 // DH, (c0 + cw) // DH):
                    q_s[b * HKV + hh // REP, pl.ds(hh % REP, 1), :] = (
                        q[b:b + 1, hh * DH - c0:(hh + 1) * DH - c0])

        def t_w2(s):
            def f():
                t = jnp.dot(h_s[:, pl.ds(s * 128, 128)], w2_v[pl.ds(s * 128, 128), :],
                            preferred_element_type=f32)
                t = (1.0 - st['gate']) * t
                if s == 0:
                    acc_s[...] = t
                else:
                    acc_s[...] += t
            return f

        def t_k(b, g, c):
            def f():
                i = b * HKV + g
                s = lax.dot_general(q_s[i].astype(bf16), k_v[b, g, pl.ds(c * KT, KT), :],
                                    (((1,), (1,)), ((), ())), preferred_element_type=f32)
                p_s[i, :, pl.ds(c * KT, KT)] = s * scale
            return f

        def t_softmax(b, g):
            def f():
                i = b * HKV + g
                s = p_s[i]
                p = jnp.exp(s - jnp.max(s, axis=-1, keepdims=True))
                l_s[i] = jnp.broadcast_to(jnp.sum(p, axis=-1, keepdims=True), (REP, DH))
                p_s[i] = p
            return f

        def t_v(b, g, c):
            def f():
                i = b * HKV + g
                o = jnp.dot(p_s[i, :, pl.ds(c * KT, KT)].astype(bf16),
                            v_v[b, g, pl.ds(c * KT, KT), :], preferred_element_type=f32)
                if c == 0:
                    o_acc[...] = o
                elif c < NKT - 1:
                    o_acc[...] += o
                else:
                    o = (o_acc[...] + o) / l_s[i]
                    for h in range(REP):
                        o_s[pl.ds(b, 1), pl.ds((g * REP + h) * DH, DH)] = o[h:h + 1, :]
            return f

        def t_wo(r, n):
            def f():
                t = jnp.dot(o_s[:, pl.ds(r, n)].astype(bf16), wo_v[pl.ds(r, n), :],
                            preferred_element_type=f32)
                acc_s[...] += st['gate'] * t
            return f

        v0 = QD - VPU_ROWS

        def t_prep():
            blk = o_s[:, pl.ds(QD - DH, DH)].astype(bf16).astype(f32) * st['gate']
            ri = lax.broadcasted_iota(jnp.int32, (VPU_ROWS, DH), 0)
            li = lax.broadcasted_iota(jnp.int32, (VPU_ROWS, DH), 1)
            sel = li == ri + (DH - VPU_ROWS)
            for b in range(B):
                col = jnp.sum(jnp.where(sel, blk[b:b + 1, :], 0.0), axis=1, keepdims=True)
                oc_s[b] = jnp.broadcast_to(col, (VPU_ROWS, DH))

        def t_vpu(r, n, last):
            def f():
                w = wo_v[pl.ds(r, n), :].astype(f32)
                for b in range(B):
                    c = oc_s[b, pl.ds(r - v0, n), :]
                    pr = w * jnp.concatenate([c] * (D // DH), axis=1)
                    a8 = pr[0:8]
                    for k in range(8, n, 8):
                        a8 = a8 + pr[k:k + 8]
                    st[('v8', b)] = a8 + st[('v8', b)] if ('v8', b) in st else a8
                if last:
                    t = jnp.concatenate(
                        [jnp.sum(st[('v8', b)], axis=0, keepdims=True) for b in range(B)], axis=0)
                    out_v[...] = (acc_s[...] + t).astype(bf16)
            return f

        tasks = []

        def add(name, ready, deps, cost, fn):
            tasks.append(dict(name=name, ready=ready, deps=deps, cost=cost, fn=fn))

        add('init', 0, [], 100, t_init)
        for key, w_v, acc, fin, width in (('w1', w1_v, h_acc, fin_h, F), ('wq', wq_v, q_acc, fin_q, QD)):
            cw = width // NSP
            for s in range(NS):
                for c in range(NSP):
                    add((key, s, c), ready_of(key, s * 128, s * 128 + 128),
                        ['init'] + ([(key, s - 1, c)] if s else []), 290,
                        t_proj(s, c * cw, cw, w_v, acc, fin))
        w1_done = [('w1', NS - 1, c) for c in range(NSP)]
        wq_done = [('wq', NS - 1, c) for c in range(NSP)]
        for (b, g) in heads:
            for c in range(NKT):
                add(('k', b, g, c), ready_of(('k', b, g), c * KT, (c + 1) * KT), wq_done, 200,
                    t_k(b, g, c))
            add(('sm', b, g), 0, [('k', b, g, c) for c in range(NKT)], 200, t_softmax(b, g))
        prev = []
        for (b, g) in heads:
            for c in range(NKT):
                add(('v', b, g, c), ready_of(('v', b, g), c * KT, (c + 1) * KT),
                    [('sm', b, g)] + prev, 200, t_v(b, g, c))
                prev = [('v', b, g, c)]
        prev = []
        for s in range(F // 128):
            add(('w2', s), ready_of('w2', s * 128, s * 128 + 128), w1_done + prev, 250, t_w2(s))
            prev = [('w2', s)]
        v_done = lambda g: [('v', b, g, NKT - 1) for b in range(B)]
        add('prep', 0, v_done(HKV - 1), 150, t_prep)
        wo_parts = [(r, 128) for r in range(0, QD - 128, 128)] + [(QD - 128, 128 - VPU_ROWS)]
        prev = [('w2', 0)]
        for ready, r, n in sorted((ready_of('wo', r, r + n), r, n) for (r, n) in wo_parts):
            add(('wo', r), ready, v_done(r // (REP * DH)) + prev, 250, t_wo(r, n))
            prev = [('wo', r)]
        acc_done = prev + [('w2', F // 128 - 1)]
        vpu_parts = ([(r, VPU_CHUNK) for r in range(v0, QD - LAST_ROWS, VPU_CHUNK)]
                     + [(r, LAST_CHUNK) for r in range(QD - LAST_ROWS, QD, LAST_CHUNK)])
        prev = ['prep']
        for (r, n) in vpu_parts:
            last = r + n == QD
            add(('vpu', r), ready_of('wo', r, r + n), prev + (acc_done if last else []), 60,
                t_vpu(r, n, last))
            prev = [('vpu', r)]

        done = set()

        def run_ready(period, budget):
            spent, progress = 0, True
            while progress:
                progress = False
                for t in tasks:
                    if t['ready'] <= period and all(d in done for d in t['deps']):
                        if spent and spent + t['cost'] > budget:
                            continue
                        t['fn']()
                        done.add(t['name'])
                        tasks.remove(t)
                        spent += t['cost']
                        progress = True
                        break

        n_periods = max(NB, NF - EARLY)
        for j in range(n_periods):
            if j < NB:
                cp_b(j).wait()
                if j + W_BG < NB:
                    cp_b(j + W_BG).start(priority=1)
            for jj in (range(EARLY + 1) if j == 0 else [j + EARLY]):
                if jj < NF:
                    cp_f(jj).wait()
            if j + W_FG < NF:
                cp_f(j + W_FG).start(priority=0)
            run_ready(j, BUDGET if j < n_periods - 1 else 10 ** 9)
        assert not tasks
        co = pltpu.make_async_copy(out_v, o_hbm, sem_m.at[0])
        co.start()
        co.wait()

    hbm = pl.BlockSpec(memory_space=pl.ANY)
    out = pl.pallas_call(
        kernel,
        out_shape=jax.ShapeDtypeStruct((B, D), bf16),
        in_specs=[hbm] * 8,
        out_specs=hbm,
        scratch_shapes=[
            pltpu.VMEM((B, D), bf16),
            pltpu.VMEM((D,), bf16),
            pltpu.VMEM((D, QD), bf16),
            pltpu.VMEM((B, HKV, W, DH), bf16),
            pltpu.VMEM((B, HKV, W, DH), bf16),
            pltpu.VMEM((QD, D), bf16),
            pltpu.VMEM((D, F), bf16),
            pltpu.VMEM((F, D), bf16),
            pltpu.VMEM((B, F), f32),
            pltpu.VMEM((B, F), bf16),
            pltpu.VMEM((B, QD), f32),
            pltpu.VMEM((B * HKV, REP, DH), f32),
            pltpu.VMEM((B * HKV, REP, W), f32),
            pltpu.VMEM((B * HKV, REP, DH), f32),
            pltpu.VMEM((REP, DH), f32),
            pltpu.VMEM((B, QD), f32),
            pltpu.VMEM((B, D), f32),
            pltpu.VMEM((B, VPU_ROWS, DH), f32),
            pltpu.VMEM((B, D), bf16),
            pltpu.SemaphoreType.DMA((W_FG,)),
            pltpu.SemaphoreType.DMA((W_BG,)),
            pltpu.SemaphoreType.DMA((2,)),
        ],
        compiler_params=pltpu.CompilerParams(
            vmem_limit_bytes=100 * 1024 * 1024,
            disable_semaphore_checks=True,
        ),
    )(A_x.reshape(B, D), A_k_cache, A_v_cache, A_wq, A_wo, B_w1, B_w2, gate_w)
    return out.reshape(B, 1, D)
```

```python
import jax
import jax.numpy as jnp
from jax import lax
import jax.experimental.pallas as pl
import jax.experimental.pallas.tpu as pltpu

HQ, DH = 32, 128
W_FG = 16
W_BG = 16
EARLY = 4
BG_BYTES = 64 * 1024
FG_BYTES = 32 * 1024
G_X = 8
G_O = 8
G_2 = 7
WO_FG = 16
WO_SEQ = 128
KT = 1024
NSP = 2
VPU_ROWS = 64
VPU_CHUNK = 32
LAST_ROWS = 32
LAST_CHUNK = 16
BUDGET = 500
PERIOD = 190
COOL = 1
URGENT = 40


@jax.jit
def pallas_gated_mix__sliding_block_cached__dense_activation_silu__decode_kernel(
    A_x: jax.Array,
    A_k_cache: jax.Array,
    A_v_cache: jax.Array,
    A_wq: jax.Array,
    A_wo: jax.Array,
    B_x: jax.Array,
    B_w1: jax.Array,
    B_w2: jax.Array,
    gate_w: jax.Array,
):
    del B_x
    B, _, D = A_x.shape
    HKV, Sk = A_k_cache.shape[1], A_k_cache.shape[2]
    F = B_w1.shape[1]
    REP = HQ // HKV
    QD = HQ * DH
    W = min(4096, max(256, Sk // 4))
    scale = DH ** -0.5
    NKT = W // KT
    NS = D // 128
    bf16, f32 = jnp.bfloat16, jnp.float32
    heads = [(b, g) for g in range(HKV) for b in range(B)]
    RX, RO, R2 = D // G_X, QD // G_O, F // G_2
    PX = 128 // G_X

    def kernel(x_hbm, k_hbm, v_hbm, wq_hbm, wo_hbm, w1_hbm, w2_hbm, g_hbm, o_hbm,
               x_v, g_v, wq_v, k_v, v_v, wo_v, w1_v, w2_v,
               xp_s, h_acc, q_acc, h_s, q_s, p_s, l_s, o_acc, o_s, acc_s, oc_s, out_v,
               sem_f, sem_b, sem_m):
        def blocks(key, src, dst, r_lo, r_hi, cw):
            G, _, C = src.shape
            return [(src.at[:, pl.ds(r, 8), pl.ds(c, cw)], dst.at[:, pl.ds(r, 8), pl.ds(c, cw)],
                     key, (0, G), (r, r + 8), (c, c + cw))
                    for r in range(r_lo, r_hi, 8) for c in range(0, C, cw)]

        def seq(key, src, dst, g, r_lo, r_hi, n):
            return [(src.at[g, pl.ds(r, n), :], dst.at[g, pl.ds(r, n), :],
                     key, (g, g + 1), (r, r + n), (0, src.shape[2]))
                    for r in range(r_lo, r_hi, n)]

        def kv_blocks(key, src, dst):
            n = BG_BYTES // (B * HKV * DH * 2)
            return [(src.at[:, :, pl.ds(Sk - W + r, n), :], dst.at[:, :, pl.ds(r, n), :],
                     key, (0, 1), (r, r + n), (0, DH)) for r in range(0, W, n)]

        bg = (blocks('wq', wq_hbm, wq_v, 0, RX, BG_BYTES // (G_X * 16))
              + kv_blocks('k', k_hbm, k_v) + kv_blocks('v', v_hbm, v_v)
              + blocks('wo', wo_hbm, wo_v, WO_FG, RO - WO_SEQ, BG_BYTES // (G_O * 16)))
        for g in range(G_O):
            bg += seq('wo', wo_hbm, wo_v, g, RO - WO_SEQ,
                      RO - (LAST_ROWS if g == G_O - 1 else 0), 32)
        bg += seq('wo', wo_hbm, wo_v, G_O - 1, RO - LAST_ROWS, RO, LAST_CHUNK)
        fg = (blocks('w1', w1_hbm, w1_v, 0, RX, FG_BYTES // (G_X * 16))
              + blocks('wo', wo_hbm, wo_v, 0, WO_FG, FG_BYTES // (G_O * 16))
              + blocks('w2', w2_hbm, w2_v, 0, R2, 256))
        NB, NF = len(bg), len(fg)
        n_periods = max(NB, NF - EARLY)

        def ready_of(key, reg=None, rws=None, cols=None):
            ov = lambda a, b: b is None or (a[0] < b[1] and a[1] > b[0])
            hit = lambda e: e[2] == key and ov(e[3], reg) and ov(e[4], rws) and ov(e[5], cols)
            return max([0] + [j for j, e in enumerate(bg) if hit(e)]
                       + [j - EARLY for j, e in enumerate(fg) if hit(e)])

        def cp_b(j):
            return pltpu.make_async_copy(bg[j][0], bg[j][1], sem_b.at[j % W_BG])

        def cp_f(j):
            return pltpu.make_async_copy(fg[j][0], fg[j][1], sem_f.at[j % W_FG])

        cx = pltpu.make_async_copy(x_hbm, x_v, sem_m.at[0])
        cg = pltpu.make_async_copy(g_hbm, g_v, sem_m.at[1])
        cx.start(priority=0)
        cg.start(priority=0)
        for j in range(W_BG):
            cp_b(j).start(priority=1)
        for j in range(W_FG):
            cp_f(j).start(priority=0)

        st = {'next_ok': 0}

        def t_init():
            cx.wait()
            cg.wait()
            xf = x_v[...].astype(f32)
            gw = g_v[...].astype(f32).reshape(1, D)
            st['gate'] = jax.nn.sigmoid(jnp.sum(xf * gw, axis=-1, keepdims=True))
            xp_s[...] = jnp.concatenate(
                [xf[:, g * RX + t * PX:g * RX + (t + 1) * PX]
                 for t in range(NS) for g in range(G_X)], axis=1).astype(bf16)

        def t_proj(t, c0, cw, w_v, acc, fin):
            def f():
                w = w_v[:, pl.ds(t * PX, PX), pl.ds(c0, cw)].reshape(128, cw)
                y = jnp.dot(xp_s[:, pl.ds(t * 128, 128)], w, preferred_element_type=f32)
                if t == 0:
                    acc[:, pl.ds(c0, cw)] = y
                elif t < NS - 1:
                    acc[:, pl.ds(c0, cw)] += y
                else:
                    fin(acc[:, pl.ds(c0, cw)] + y, c0, cw)
            return f

        def fin_h(h, c0, cw):
            h_s[:, pl.ds(c0, cw)] = (h * jax.nn.sigmoid(h)).astype(bf16)

        def fin_q(q, c0, cw):
            for b in range(B):
                for hh in range(c0 // DH, (c0 + cw) // DH):
                    q_s[b * HKV + hh // REP, pl.ds(hh % REP, 1), :] = (
                        q[b:b + 1, hh * DH - c0:(hh + 1) * DH - c0])

        def t_w2(g, r, first):
            def f():
                t = jnp.dot(h_s[:, pl.ds(g * R2 + r, 128)], w2_v[g, pl.ds(r, 128), :],
                            preferred_element_type=f32)
                t = (1.0 - st['gate']) * t
                if first:
                    acc_s[...] = t
                else:
                    acc_s[...] += t
            return f

        def t_k(b, g, c):
            def f():
                i = b * HKV + g
                s = lax.dot_general(q_s[i].astype(bf16), k_v[b, g, pl.ds(c * KT, KT), :],
                                    (((1,), (1,)), ((), ())), preferred_element_type=f32)
                p_s[i, :, pl.ds(c * KT, KT)] = s * scale
            return f

        def t_softmax(b, g):
            def f():
                i = b * HKV + g
                s = p_s[i]
                p = jnp.exp(s - jnp.max(s, axis=-1, keepdims=True))
                l_s[i] = jnp.broadcast_to(jnp.sum(p, axis=-1, keepdims=True), (REP, DH))
                p_s[i] = p
            return f

        def t_v(b, g, c):
            def f():
                i = b * HKV + g
                o = jnp.dot(p_s[i, :, pl.ds(c * KT, KT)].astype(bf16),
                            v_v[b, g, pl.ds(c * KT, KT), :], preferred_element_type=f32)
                if c == 0:
                    o_acc[i] = o
                elif c < NKT - 1:
                    o_acc[i] += o
                else:
                    o = (o_acc[i] + o) / l_s[i]
                    for h in range(REP):
                        o_s[pl.ds(b, 1), pl.ds((g * REP + h) * DH, DH)] = o[h:h + 1, :]
            return f

        def t_wo(g, r, n):
            def f():
                t = jnp.dot(o_s[:, pl.ds(g * RO + r, n)].astype(bf16), wo_v[g, pl.ds(r, n), :],
                            preferred_element_type=f32)
                acc_s[...] += st['gate'] * t
            return f

        v0 = RO - VPU_ROWS

        def t_prep():
            blk = o_s[:, pl.ds(QD - DH, DH)].astype(bf16).astype(f32) * st['gate']
            ri = lax.broadcasted_iota(jnp.int32, (VPU_ROWS, DH), 0)
            li = lax.broadcasted_iota(jnp.int32, (VPU_ROWS, DH), 1)
            sel = li == ri + (DH - VPU_ROWS)
            for b in range(B):
                col = jnp.sum(jnp.where(sel, blk[b:b + 1, :], 0.0), axis=1, keepdims=True)
                oc_s[b] = jnp.broadcast_to(col, (VPU_ROWS, DH))

        def t_vpu(r, n, last):
            def f():
                w = wo_v[G_O - 1, pl.ds(r, n), :].astype(f32)
                for b in range(B):
                    c = oc_s[b, pl.ds(r - v0, n), :]
                    pr = w * jnp.concatenate([c] * (D // DH), axis=1)
                    a8 = pr[0:8]
                    for k in range(8, n, 8):
                        a8 = a8 + pr[k:k + 8]
                    st[('v8', b)] = a8 + st[('v8', b)] if ('v8', b) in st else a8
                if last:
                    t = jnp.concatenate(
                        [jnp.sum(st[('v8', b)], axis=0, keepdims=True) for b in range(B)], axis=0)
                    out_v[...] = (acc_s[...] + t).astype(bf16)
            return f

        tasks = []

        def add(name, ready, deps, cost, fn):
            tasks.append(dict(name=name, ready=ready, deps=deps, cost=cost, fn=fn))

        add('init', 0, [], 100, t_init)
        for key, w_v, acc, fin, width in (('w1', w1_v, h_acc, fin_h, F), ('wq', wq_v, q_acc, fin_q, QD)):
            cw = width // NSP
            for t in range(NS):
                for c in range(NSP):
                    add((key, t, c),
                        ready_of(key, rws=(t * PX, (t + 1) * PX), cols=(c * cw, (c + 1) * cw)),
                        ['init'] + ([(key, t - 1, c)] if t else []), 290,
                        t_proj(t, c * cw, cw, w_v, acc, fin))
        w1_done = [('w1', NS - 1, c) for c in range(NSP)]
        wq_done = [('wq', NS - 1, c) for c in range(NSP)]
        for c in range(NKT):
            for (b, g) in heads:
                add(('k', b, g, c), ready_of('k', rws=(c * KT, (c + 1) * KT)), wq_done, 200,
                    t_k(b, g, c))
        for (b, g) in heads:
            add(('sm', b, g), 0, [('k', b, g, c) for c in range(NKT)], 200, t_softmax(b, g))
        for c in range(NKT):
            for (b, g) in heads:
                add(('v', b, g, c), ready_of('v', rws=(c * KT, (c + 1) * KT)),
                    [('sm', b, g)] + ([('v', b, g, c - 1)] if c else []), 200, t_v(b, g, c))
        prev = []
        for r in range(0, R2, 128):
            for g in range(G_2):
                add(('w2', g, r), ready_of('w2', rws=(r, r + 128)), w1_done + prev, 250,
                    t_w2(g, r, not prev))
                prev = [('w2', g, r)]
        w2_last = prev
        v_done = lambda g: [('v', b, g, NKT - 1) for b in range(B)]
        add('prep', 0, v_done(HKV - 1), 150, t_prep)
        wo_parts = [(g, r, 128) for g in range(G_O) for r in range(0, RO, 128)]
        wo_parts[-1] = (G_O - 1, RO - 128, 128 - VPU_ROWS)
        prev = [('w2', 0, 0)]
        for ready, g, r, n in sorted((ready_of('wo', reg=(g, g + 1), rws=(r, r + n)), g, r, n)
                                     for (g, r, n) in wo_parts):
            add(('wo', g, r), ready, v_done((g * RO + r) // (REP * DH)) + prev, 250, t_wo(g, r, n))
            prev = [('wo', g, r)]
        acc_done = prev + w2_last
        vpu_parts = ([(r, VPU_CHUNK) for r in range(v0, RO - LAST_ROWS, VPU_CHUNK)]
                     + [(r, LAST_CHUNK) for r in range(RO - LAST_ROWS, RO, LAST_CHUNK)])
        prev = ['prep']
        for (r, n) in vpu_parts:
            last = r + n == RO
            add(('vpu', r), ready_of('wo', reg=(G_O - 1, G_O), rws=(r, r + n)),
                prev + (acc_done if last else []), 60, t_vpu(r, n, last))
            prev = [('vpu', r)]

        done = set()

        def run_ready(period, budget):
            if period < st['next_ok'] and period < n_periods - URGENT:
                return
            spent, progress = 0, True
            while progress:
                progress = False
                for t in tasks:
                    if t['ready'] <= period and all(d in done for d in t['deps']):
                        if spent and spent + t['cost'] > budget:
                            continue
                        t['fn']()
                        done.add(t['name'])
                        tasks.remove(t)
                        spent += t['cost']
                        est = 150 + spent * 0.3 if spent > t['cost'] else t['cost']
                        st['next_ok'] = period + int(-(-est // PERIOD)) + COOL
                        progress = True
                        break

        for j in range(n_periods):
            if j < NB:
                cp_b(j).wait()
                if j + W_BG < NB:
                    cp_b(j + W_BG).start(priority=1)
            for jj in (range(EARLY + 1) if j == 0 else [j + EARLY]):
                if jj < NF:
                    cp_f(jj).wait()
            if j + W_FG < NF:
                cp_f(j + W_FG).start(priority=0)
            run_ready(j, BUDGET if j < n_periods - 1 else 10 ** 9)
        assert not tasks
        co = pltpu.make_async_copy(out_v, o_hbm, sem_m.at[0])
        co.start()
        co.wait()

    hbm = pl.BlockSpec(memory_space=pl.ANY)
    out = pl.pallas_call(
        kernel,
        out_shape=jax.ShapeDtypeStruct((B, D), bf16),
        in_specs=[hbm] * 8,
        out_specs=hbm,
        scratch_shapes=[
            pltpu.VMEM((B, D), bf16),
            pltpu.VMEM((D,), bf16),
            pltpu.VMEM((G_X, RX, QD), bf16),
            pltpu.VMEM((B, HKV, W, DH), bf16),
            pltpu.VMEM((B, HKV, W, DH), bf16),
            pltpu.VMEM((G_O, RO, D), bf16),
            pltpu.VMEM((G_X, RX, F), bf16),
            pltpu.VMEM((G_2, R2, D), bf16),
            pltpu.VMEM((B, D), bf16),
            pltpu.VMEM((B, F), f32),
            pltpu.VMEM((B, QD), f32),
            pltpu.VMEM((B, F), bf16),
            pltpu.VMEM((B * HKV, REP, DH), f32),
            pltpu.VMEM((B * HKV, REP, W), f32),
            pltpu.VMEM((B * HKV, REP, DH), f32),
            pltpu.VMEM((B * HKV, REP, DH), f32),
            pltpu.VMEM((B, QD), f32),
            pltpu.VMEM((B, D), f32),
            pltpu.VMEM((B, VPU_ROWS, DH), f32),
            pltpu.VMEM((B, D), bf16),
            pltpu.SemaphoreType.DMA((W_FG,)),
            pltpu.SemaphoreType.DMA((W_BG,)),
            pltpu.SemaphoreType.DMA((2,)),
        ],
        compiler_params=pltpu.CompilerParams(
            vmem_limit_bytes=100 * 1024 * 1024,
            disable_semaphore_checks=True,
        ),
    )(A_x.reshape(B, D), A_k_cache, A_v_cache, A_wq.reshape(G_X, RX, QD),
      A_wo.reshape(G_O, RO, D), B_w1.reshape(G_X, RX, F), B_w2.reshape(G_2, R2, D), gate_w)
    return out.reshape(B, 1, D)
```

```python
import jax
import jax.numpy as jnp
from jax import lax
import jax.experimental.pallas as pl
import jax.experimental.pallas.tpu as pltpu

HQ, DH = 32, 128
W_FG = 32
W_BG = 32
EARLY = 8
BG_BYTES = 32 * 1024
FG_BYTES = 16 * 1024
G_X = 8
G_O = 8
G_2 = 7
WO_SEQ = 128
KT = 1024
NSP = 2
VPU_ROWS = 64
VPU_CHUNK = 32
LAST_ROWS = 32
LAST_CHUNK = 16
BUDGET = 500
PERIOD = 95
COOL = 2
URGENT = 80


@jax.jit
def pallas_gated_mix__sliding_block_cached__dense_activation_silu__decode_kernel(
    A_x: jax.Array,
    A_k_cache: jax.Array,
    A_v_cache: jax.Array,
    A_wq: jax.Array,
    A_wo: jax.Array,
    B_x: jax.Array,
    B_w1: jax.Array,
    B_w2: jax.Array,
    gate_w: jax.Array,
):
    del B_x
    B, _, D = A_x.shape
    HKV, Sk = A_k_cache.shape[1], A_k_cache.shape[2]
    F = B_w1.shape[1]
    REP = HQ // HKV
    QD = HQ * DH
    W = min(4096, max(256, Sk // 4))
    scale = DH ** -0.5
    NKT = W // KT
    NS = D // 128
    bf16, f32 = jnp.bfloat16, jnp.float32
    heads = [(b, g) for g in range(HKV) for b in range(B)]
    RX, RO, R2 = D // G_X, QD // G_O, F // G_2
    PX = 128 // G_X

    def kernel(x_hbm, k_hbm, v_hbm, wq_hbm, wo_hbm, w1_hbm, w2_hbm, g_hbm, o_hbm,
               x_v, g_v, wq_v, k_v, v_v, wo_v, w1_v, w2_v,
               xp_s, h_acc, q_acc, h_s, q_s, p_s, l_s, o_acc, o_s, acc_s, oc_s, out_v,
               sem_f, sem_b, sem_m):
        def blocks(key, src, dst, r_lo, r_hi, cw):
            G, _, C = src.shape
            return [(src.at[:, pl.ds(r, 8), pl.ds(c, cw)], dst.at[:, pl.ds(r, 8), pl.ds(c, cw)],
                     key, (0, G), (r, r + 8), (c, c + cw))
                    for r in range(r_lo, r_hi, 8) for c in range(0, C, cw)]

        def seq(key, src, dst, g, r_lo, r_hi, n):
            return [(src.at[g, pl.ds(r, n), :], dst.at[g, pl.ds(r, n), :],
                     key, (g, g + 1), (r, r + n), (0, src.shape[2]))
                    for r in range(r_lo, r_hi, n)]

        def kv_blocks(key, src, dst):
            n = BG_BYTES // (B * HKV * DH * 2)
            return [(src.at[:, :, pl.ds(Sk - W + r, n), :], dst.at[:, :, pl.ds(r, n), :],
                     key, (0, 1), (r, r + n), (0, DH)) for r in range(0, W, n)]

        bg = (blocks('wq', wq_hbm, wq_v, 0, RX, BG_BYTES // (G_X * 16))
              + kv_blocks('k', k_hbm, k_v) + kv_blocks('v', v_hbm, v_v)
              + blocks('wo', wo_hbm, wo_v, 0, RO - WO_SEQ, BG_BYTES // (G_O * 16)))
        for g in range(G_O):
            bg += seq('wo', wo_hbm, wo_v, g, RO - WO_SEQ,
                      RO - (LAST_ROWS if g == G_O - 1 else 0), 32)
        bg += seq('wo', wo_hbm, wo_v, G_O - 1, RO - LAST_ROWS, RO, LAST_CHUNK)
        fg = (blocks('w1', w1_hbm, w1_v, 0, RX, FG_BYTES // (G_X * 16))
              + blocks('w2', w2_hbm, w2_v, 0, R2, 128))
        NB, NF = len(bg), len(fg)
        n_periods = max(NB, NF - EARLY)

        def ready_of(key, reg=None, rws=None, cols=None):
            ov = lambda a, b: b is None or (a[0] < b[1] and a[1] > b[0])
            hit = lambda e: e[2] == key and ov(e[3], reg) and ov(e[4], rws) and ov(e[5], cols)
            return max([0] + [j for j, e in enumerate(bg) if hit(e)]
                       + [j - EARLY for j, e in enumerate(fg) if hit(e)])

        def cp_b(j):
            return pltpu.make_async_copy(bg[j][0], bg[j][1], sem_b.at[j % W_BG])

        def cp_f(j):
            return pltpu.make_async_copy(fg[j][0], fg[j][1], sem_f.at[j % W_FG])

        cx = pltpu.make_async_copy(x_hbm, x_v, sem_m.at[0])
        cg = pltpu.make_async_copy(g_hbm, g_v, sem_m.at[1])
        cx.start(priority=0)
        cg.start(priority=0)
        for j in range(W_BG):
            cp_b(j).start(priority=1)
        for j in range(W_FG):
            cp_f(j).start(priority=0)

        st = {'next_ok': 0}

        def t_init():
            cx.wait()
            cg.wait()
            xf = x_v[...].astype(f32)
            gw = g_v[...].astype(f32).reshape(1, D)
            st['gate'] = jax.nn.sigmoid(jnp.sum(xf * gw, axis=-1, keepdims=True))
            xp_s[...] = jnp.concatenate(
                [xf[:, g * RX + t * PX:g * RX + (t + 1) * PX]
                 for t in range(NS) for g in range(G_X)], axis=1).astype(bf16)

        def t_proj(t, c0, cw, w_v, acc, fin):
            def f():
                w = w_v[:, pl.ds(t * PX, PX), pl.ds(c0, cw)].reshape(128, cw)
                y = jnp.dot(xp_s[:, pl.ds(t * 128, 128)], w, preferred_element_type=f32)
                if t == 0:
                    acc[:, pl.ds(c0, cw)] = y
                elif t < NS - 1:
                    acc[:, pl.ds(c0, cw)] += y
                else:
                    fin(acc[:, pl.ds(c0, cw)] + y, c0, cw)
            return f

        def fin_h(h, c0, cw):
            h_s[:, pl.ds(c0, cw)] = (h * jax.nn.sigmoid(h)).astype(bf16)

        def fin_q(q, c0, cw):
            for b in range(B):
                for hh in range(c0 // DH, (c0 + cw) // DH):
                    q_s[b * HKV + hh // REP, pl.ds(hh % REP, 1), :] = (
                        q[b:b + 1, hh * DH - c0:(hh + 1) * DH - c0])

        def t_w2(g, r, first):
            def f():
                t = jnp.dot(h_s[:, pl.ds(g * R2 + r, 128)], w2_v[g, pl.ds(r, 128), :],
                            preferred_element_type=f32)
                t = (1.0 - st['gate']) * t
                if first:
                    acc_s[...] = t
                else:
                    acc_s[...] += t
            return f

        def t_k(b, g, c):
            def f():
                i = b * HKV + g
                s = lax.dot_general(q_s[i].astype(bf16), k_v[b, g, pl.ds(c * KT, KT), :],
                                    (((1,), (1,)), ((), ())), preferred_element_type=f32)
                p_s[i, :, pl.ds(c * KT, KT)] = s * scale
            return f

        def t_softmax(b, g):
            def f():
                i = b * HKV + g
                s = p_s[i]
                p = jnp.exp(s - jnp.max(s, axis=-1, keepdims=True))
                l_s[i] = jnp.broadcast_to(jnp.sum(p, axis=-1, keepdims=True), (REP, DH))
                p_s[i] = p
            return f

        def t_v(b, g, c):
            def f():
                i = b * HKV + g
                o = jnp.dot(p_s[i, :, pl.ds(c * KT, KT)].astype(bf16),
                            v_v[b, g, pl.ds(c * KT, KT), :], preferred_element_type=f32)
                if c == 0:
                    o_acc[i] = o
                elif c < NKT - 1:
                    o_acc[i] += o
                else:
                    o = (o_acc[i] + o) / l_s[i]
                    for h in range(REP):
                        o_s[pl.ds(b, 1), pl.ds((g * REP + h) * DH, DH)] = o[h:h + 1, :]
            return f

        def t_wo(g, r, n):
            def f():
                t = jnp.dot(o_s[:, pl.ds(g * RO + r, n)].astype(bf16), wo_v[g, pl.ds(r, n), :],
                            preferred_element_type=f32)
                acc_s[...] += st['gate'] * t
            return f

        v0 = RO - VPU_ROWS

        def t_prep():
            blk = o_s[:, pl.ds(QD - DH, DH)].astype(bf16).astype(f32) * st['gate']
            ri = lax.broadcasted_iota(jnp.int32, (VPU_ROWS, DH), 0)
            li = lax.broadcasted_iota(jnp.int32, (VPU_ROWS, DH), 1)
            sel = li == ri + (DH - VPU_ROWS)
            for b in range(B):
                col = jnp.sum(jnp.where(sel, blk[b:b + 1, :], 0.0), axis=1, keepdims=True)
                oc_s[b] = jnp.broadcast_to(col, (VPU_ROWS, DH))

        def t_vpu(r, n, last):
            def f():
                w = wo_v[G_O - 1, pl.ds(r, n), :].astype(f32)
                for b in range(B):
                    c = oc_s[b, pl.ds(r - v0, n), :]
                    pr = w * jnp.concatenate([c] * (D // DH), axis=1)
                    a8 = pr[0:8]
                    for k in range(8, n, 8):
                        a8 = a8 + pr[k:k + 8]
                    st[('v8', b)] = a8 + st[('v8', b)] if ('v8', b) in st else a8
                if last:
                    t = jnp.concatenate(
                        [jnp.sum(st[('v8', b)], axis=0, keepdims=True) for b in range(B)], axis=0)
                    out_v[...] = (acc_s[...] + t).astype(bf16)
            return f

        tasks = []

        def add(name, ready, deps, cost, fn):
            tasks.append(dict(name=name, ready=ready, deps=deps, cost=cost, fn=fn))

        add('init', 0, [], 100, t_init)
        for key, w_v, acc, fin, width in (('w1', w1_v, h_acc, fin_h, F), ('wq', wq_v, q_acc, fin_q, QD)):
            cw = width // NSP
            for t in range(NS):
                for c in range(NSP):
                    add((key, t, c),
                        ready_of(key, rws=(t * PX, (t + 1) * PX), cols=(c * cw, (c + 1) * cw)),
                        ['init'] + ([(key, t - 1, c)] if t else []), 290,
                        t_proj(t, c * cw, cw, w_v, acc, fin))
        w1_done = [('w1', NS - 1, c) for c in range(NSP)]
        wq_done = [('wq', NS - 1, c) for c in range(NSP)]
        for c in range(NKT):
            for (b, g) in heads:
                add(('k', b, g, c), ready_of('k', rws=(c * KT, (c + 1) * KT)), wq_done, 200,
                    t_k(b, g, c))
        for (b, g) in heads:
            add(('sm', b, g), 0, [('k', b, g, c) for c in range(NKT)], 200, t_softmax(b, g))
        for c in range(NKT):
            for (b, g) in heads:
                add(('v', b, g, c), ready_of('v', rws=(c * KT, (c + 1) * KT)),
                    [('sm', b, g)] + ([('v', b, g, c - 1)] if c else []), 200, t_v(b, g, c))
        prev = []
        for r in range(0, R2, 128):
            for g in range(G_2):
                add(('w2', g, r), ready_of('w2', rws=(r, r + 128)), w1_done + prev, 250,
                    t_w2(g, r, not prev))
                prev = [('w2', g, r)]
        w2_last = prev
        v_done = lambda g: [('v', b, g, NKT - 1) for b in range(B)]
        add('prep', 0, v_done(HKV - 1), 150, t_prep)
        wo_parts = [(g, r, 128) for g in range(G_O) for r in range(0, RO, 128)]
        wo_parts[-1] = (G_O - 1, RO - 128, 128 - VPU_ROWS)
        prev = [('w2', 0, 0)]
        for ready, g, r, n in sorted((ready_of('wo', reg=(g, g + 1), rws=(r, r + n)), g, r, n)
                                     for (g, r, n) in wo_parts):
            add(('wo', g, r), ready, v_done((g * RO + r) // (REP * DH)) + prev, 250, t_wo(g, r, n))
            prev = [('wo', g, r)]
        acc_done = prev + w2_last
        vpu_parts = ([(r, VPU_CHUNK) for r in range(v0, RO - LAST_ROWS, VPU_CHUNK)]
                     + [(r, LAST_CHUNK) for r in range(RO - LAST_ROWS, RO, LAST_CHUNK)])
        prev = ['prep']
        for (r, n) in vpu_parts:
            last = r + n == RO
            add(('vpu', r), ready_of('wo', reg=(G_O - 1, G_O), rws=(r, r + n)),
                prev + (acc_done if last else []), 60, t_vpu(r, n, last))
            prev = [('vpu', r)]

        done = set()

        def run_ready(period, budget):
            if period < st['next_ok'] and period < n_periods - URGENT:
                return
            spent, progress = 0, True
            while progress:
                progress = False
                for t in tasks:
                    if t['ready'] <= period and all(d in done for d in t['deps']):
                        if spent and spent + t['cost'] > budget:
                            continue
                        t['fn']()
                        done.add(t['name'])
                        tasks.remove(t)
                        spent += t['cost']
                        est = 150 + spent * 0.3 if spent > t['cost'] else t['cost']
                        st['next_ok'] = period + int(-(-est // PERIOD)) + COOL
                        progress = True
                        break

        for j in range(n_periods):
            if j < NB:
                cp_b(j).wait()
                if j + W_BG < NB:
                    cp_b(j + W_BG).start(priority=1)
            for jj in (range(EARLY + 1) if j == 0 else [j + EARLY]):
                if jj < NF:
                    cp_f(jj).wait()
            if j + W_FG < NF:
                cp_f(j + W_FG).start(priority=0)
            run_ready(j, BUDGET if j < n_periods - 1 else 10 ** 9)
        assert not tasks
        co = pltpu.make_async_copy(out_v, o_hbm, sem_m.at[0])
        co.start()
        co.wait()

    params = dict(vmem_limit_bytes=100 * 1024 * 1024)
    if hasattr(pltpu.CompilerParams, 'disable_semaphore_checks'):
        params['disable_semaphore_checks'] = True
    hbm = pl.BlockSpec(memory_space=pl.ANY)
    out = pl.pallas_call(
        kernel,
        out_shape=jax.ShapeDtypeStruct((B, D), bf16),
        in_specs=[hbm] * 8,
        out_specs=hbm,
        scratch_shapes=[
            pltpu.VMEM((B, D), bf16),
            pltpu.VMEM((D,), bf16),
            pltpu.VMEM((G_X, RX, QD), bf16),
            pltpu.VMEM((B, HKV, W, DH), bf16),
            pltpu.VMEM((B, HKV, W, DH), bf16),
            pltpu.VMEM((G_O, RO, D), bf16),
            pltpu.VMEM((G_X, RX, F), bf16),
            pltpu.VMEM((G_2, R2, D), bf16),
            pltpu.VMEM((B, D), bf16),
            pltpu.VMEM((B, F), f32),
            pltpu.VMEM((B, QD), f32),
            pltpu.VMEM((B, F), bf16),
            pltpu.VMEM((B * HKV, REP, DH), f32),
            pltpu.VMEM((B * HKV, REP, W), f32),
            pltpu.VMEM((B * HKV, REP, DH), f32),
            pltpu.VMEM((B * HKV, REP, DH), f32),
            pltpu.VMEM((B, QD), f32),
            pltpu.VMEM((B, D), f32),
            pltpu.VMEM((B, VPU_ROWS, DH), f32),
            pltpu.VMEM((B, D), bf16),
            pltpu.SemaphoreType.DMA((W_FG,)),
            pltpu.SemaphoreType.DMA((W_BG,)),
            pltpu.SemaphoreType.DMA((2,)),
        ],
        compiler_params=pltpu.CompilerParams(**params),
    )(A_x.reshape(B, D), A_k_cache, A_v_cache, A_wq.reshape(G_X, RX, QD),
      A_wo.reshape(G_O, RO, D), B_w1.reshape(G_X, RX, F), B_w2.reshape(G_2, R2, D), gate_w)
    return out.reshape(B, 1, D)
```
